```python
import os as _os
_os.environ.setdefault("JAX_PLATFORMS", "cpu")
import jax
import jax.numpy as jnp

def _softmax(x, axis=-1):
    return jax.nn.softmax(x, axis=axis)
def _gelu(x):
    return jax.nn.gelu(x, approximate=True)
def _silu(x):
    return jax.nn.silu(x)
def _sigmoid(x):
    return jax.nn.sigmoid(x)
def _layernorm(x, axis=-1, eps=1e-5):
    m = jnp.mean(x, axis=axis, keepdims=True)
    v = jnp.var(x, axis=axis, keepdims=True)
    return (x - m) / jnp.sqrt(v + eps)
def _scatter_add(tgt, idx, src, axis=0):
    return tgt.at[idx].add(src)
def _segment_sum(src, seg, n):
    return jax.ops.segment_sum(src, seg, n)
class _Rng:
    def __init__(self, key):
        self._k = key
    def _next(self):
        self._k, sub = jax.random.split(self._k)
        return sub
    def normal(self, shape):
        return jax.random.normal(self._next(), shape, dtype=jnp.bfloat16)
    def randint(self, lo, hi, shape):
        return jax.random.randint(self._next(), shape, lo, hi, dtype=jnp.int32)
    def uniform(self, shape, lo=0.0, hi=1.0):
        return jax.random.uniform(self._next(), shape, jnp.bfloat16, lo, hi)
    def permutation(self, n):
        return jax.random.permutation(self._next(), n)


kernel_name = 'concat_heads__spectral_gfnet__mha_block__prompt'

def setup_inputs():
    _rng = _Rng(jax.random.key(int.from_bytes(__import__("os").urandom(4), "little")))
    _w = (lambda a: (lambda t: t.astype(jnp.bfloat16) if jnp.issubdtype(t.dtype, jnp.floating) else t)(jnp.asarray(a)))
    def _A_setup():
        B, S, D = 1, 2048, 576
        Df = D // 2 + 1
        return {
            "x": _w((lambda *s: _rng.normal(s) * 0.05)(B, S, D)),
            "w_r": _w((lambda *s: _rng.normal(s) * 0.05)(S, Df) * 0.02),
            "w_i": _w((lambda *s: _rng.normal(s) * 0.05)(S, Df) * 0.02),
        }
    _A_in = _A_setup()

    def _B_setup():
        B, S, D, H = 1, 2048, 576, 32
        return {
            "x": _w((lambda *s: _rng.normal(s) * 0.1)(B, S, D)),
            "wqkv": _w((lambda *s: _rng.normal(s) * 0.1)(D, 3 * D)),
            "wo": _w((lambda *s: _rng.normal(s) * 0.05)(D, D)),
        }
    _B_in = _B_setup()

    return {
        "A_x": _A_in["x"],
        "A_w_r": _A_in["w_r"],
        "A_w_i": _A_in["w_i"],
        "B_x": _B_in["x"],
        "B_wqkv": _B_in["wqkv"],
        "B_wo": _B_in["wo"],
    }

def reference(A_x, A_w_r, A_w_i, B_x, B_wqkv, B_wo):
    def _A_ref(x, w_r, w_i):
        B, S, D = x.shape
        X = (lambda x, axes=(-2,-1): jnp.fft.rfft2(x.astype(jnp.float32), axes=axes))(x, axes=(-2, -1))
        W = w_r + 1j * w_i
        X = X * W
        y = (lambda x, s, axes=(-2,-1): jnp.fft.irfft2(x, s=s, axes=axes).astype(jnp.bfloat16))(X, (S, D), axes=(-2, -1))
        return y

    def _B_ref(x, wqkv, wo):
        B, S, D = x.shape
        H = 32
        Dh = D // H
        qkv = (lambda x, *d: x.transpose(*d))((x @ wqkv).reshape(B, S, 3, H, Dh), 2, 0, 3, 1, 4)
        q, k, v = qkv[0], qkv[1], qkv[2]
        scores = jnp.einsum("bhqd,bhkd->bhqk", q, k) * (Dh ** -0.5)
        p = _softmax(scores, axis=-1)
        o = jnp.einsum("bhqk,bhkd->bhqd", p, v)
        return (lambda x, *d: x.transpose(*d))(o, 0, 2, 1, 3).reshape(B, S, D) @ wo

    a = _A_ref(A_x, A_w_r, A_w_i)
    b = _B_ref(B_x, B_wqkv, B_wo)
    return jnp.concatenate([a, b], axis=-1)
```

```python
import numpy as np
import jax
import jax.numpy as jnp
from jax import lax
import jax.experimental.pallas as pl
import jax.experimental.pallas.tpu as pltpu

F32 = jnp.float32
BF16 = jnp.bfloat16

S = 2048
D = 576
DF = D // 2 + 1
H = 32
DH = D // H
QB = 512
NQB = S // QB
NT = QB // 128
CH = 128
NCH = S // CH
G = 2
NSTEP = H // G
NV = 1
SK = 4


def _dft_consts():
    d = np.arange(D)[:, None]
    k = np.arange(DF)[None, :]
    ang = 2 * np.pi * ((d * k) % D) / D
    c = np.cos(ang)
    s = -np.sin(ang)
    fd = np.zeros((D, 640))
    fd[:, 0:256] = c[:, :256]
    fd[:, 256:512] = s[:, :256]
    fd[:, 512:512 + 33] = c[:, 256:]
    fd[:, 576:576 + 33] = s[:, 256:]
    w = np.full(DF, 2.0)
    w[0] = 1.0
    w[-1] = 1.0
    ci = (c * w[None, :]).T / D
    si = (s * w[None, :]).T / D
    si[0, :] = 0.0
    si[-1, :] = 0.0
    fdi = np.zeros((640, D))
    fdi[0:256] = ci[:256]
    fdi[256:512] = si[:256]
    fdi[512:512 + 33] = ci[256:]
    fdi[576:576 + 33] = si[256:]
    k1 = np.arange(16)[:, None, None]
    k2 = np.arange(128)[None, :, None]
    b = np.arange(128)[None, None, :]
    a = 2 * np.pi * ((b * (k1 + 16 * k2)) % S) / S
    fr = np.cos(a)
    fi = -np.sin(a)
    g = np.concatenate([np.concatenate([fr, -fi], 2), np.concatenate([fi, fr], 2)], 1)
    gr = fr.transpose(0, 2, 1) / S
    gi = -fi.transpose(0, 2, 1) / S
    ginv = np.concatenate([np.concatenate([gr, -gi], 2), np.concatenate([gi, gr], 2)], 1)
    return tuple(np.ascontiguousarray(t, dtype=np.float32) for t in (fd, fdi, g, ginv))


_FD, _FDI, _G, _GI = _dft_consts()


def _head_tile(h):
    lo = h * DH
    j = lo // 128
    if (lo + DH - 1) // 128 != j or j == 4:
        t = (lo + 64) // 128
        return t, 128 * t - 64, 128 * t
    return 5 + j, 128 * j + 64, 128 * j


def _cmul_const(re, im, c, s):
    if c == 1.0 and s == 0.0:
        return re, im
    if c == 0.0 and s == -1.0:
        return im, -re
    if c == 0.0 and s == 1.0:
        return -im, re
    if abs(abs(c) - abs(s)) < 1e-12:
        if s > 0 and c > 0:
            return (re - im) * c, (re + im) * c
        if s < 0 and c > 0:
            return (re + im) * c, (im - re) * c
        if s > 0 and c < 0:
            return (re + im) * c, (im - re) * c
        if s < 0 and c < 0:
            return (re - im) * c, (re + im) * c
    return re * c - im * s, re * s + im * c


def _fft_list(xr, xi, sign):
    n = len(xr)
    if n == 1:
        return xr, xi
    er, ei = _fft_list(xr[0::2], xi[0::2], sign)
    orr, oi = _fft_list(xr[1::2], xi[1::2], sign)
    yr = [None] * n
    yi = [None] * n
    for k in range(n // 2):
        ang = sign * 2 * np.pi * k / n
        c = float(np.round(np.cos(ang), 15))
        s = float(np.round(np.sin(ang), 15))
        tr, ti = _cmul_const(orr[k], oi[k], c, s)
        yr[k] = er[k] + tr
        yi[k] = ei[k] + ti
        yr[k + n // 2] = er[k] - tr
        yi[k + n // 2] = ei[k] - ti
    return yr, yi


def _kernel(ax_h, wr_h, wi_h, bx_h, wqkv_h, wo_h, fd_h, fdi_h, g_h, gi_h,
            out_ref,
            ax_v, wr_v, wi_v, bx_v, wqkv_v, wo_v, fd_v, fdi_v, g_v, gi_v, sems,
            kt, qm, qp, qf, kv, qbt, vt, vtp, wt,
            xr, xi, fr, fi, wrf, wif, ul,
            sa0, sa1, sb0, sb1, ma, mb, ot, ora, orb):
    i = pl.program_id(0)

    def cp(n, src, dst):
        return pltpu.make_async_copy(src, dst, sems.at[n])

    NR = S // 512
    def chunk_cp(which, r):
        src, dst = ((ax_h, ax_v), (wr_h, wr_v), (wi_h, wi_v))[which]
        c0 = r * 512 if isinstance(r, int) else pl.multiple_of(r * 512, 512)
        return cp(which * NR + r, src.at[:, pl.ds(c0, 512)], dst.at[:, pl.ds(c0, 512)])

    fd_cp, wqkv_cp, bx_cp, g_cp, gi_cp, wo_cp, fdi_cp = [
        cp(3 * NR + n, src, dst) for n, (src, dst) in enumerate((
            (fd_h, fd_v), (wqkv_h, wqkv_v), (bx_h, bx_v),
            (g_h, g_v), (gi_h, gi_v), (wo_h, wo_v), (fdi_h, fdi_v)))]

    scale = float(DH ** -0.5 * np.log2(np.e))
    TN = (((0,), (0,)), ((), ()))

    @pl.when(i == 0)
    def _setup():
        fd_cp.start()
        for r in range(NR):
            for which in range(3):
                chunk_cp(which, r).start()
        for c in (wqkv_cp, bx_cp, g_cp, gi_cp, wo_cp, fdi_cp):
            c.start()
        ot[...] = jnp.zeros((D, QB), F32)
        orb[...] = jnp.ones(orb.shape, F32)
        fd_cp.wait()

        def wconv(c0, t, which):
            src, dst = ((wr_v, wrf), (wi_v, wif))[which]
            if t < 2:
                w = src[t * 128:(t + 1) * 128, pl.ds(c0, 128)].astype(F32)
            else:
                w = jnp.concatenate([src[256:DF, pl.ds(c0, 128)].astype(F32),
                                     jnp.zeros((384 - DF, 128), F32)], axis=0)
            dst[t, pl.ds(c0, 128), :] = w.T

        def ph1(r, carry):
            for which in range(3):
                chunk_cp(which, r).wait()
            for u in range(4):
                ru = pl.multiple_of(r * 512 + u * 128, 128)
                x1 = lax.dot_general(ax_v[:, pl.ds(ru, 128)], fd_v[...], TN, preferred_element_type=F32)
                for t in range(2):
                    xr[t, pl.ds(ru, 128), :] = x1[:, t * 128:(t + 1) * 128]
                    xi[t, pl.ds(ru, 128), :] = x1[:, 256 + t * 128:256 + (t + 1) * 128]
                tail = x1[:, 512:640]
                xr[2, pl.ds(ru, 128), :] = tail
                xi[2, pl.ds(ru, 128), :] = pltpu.roll(tail, 64, 1)
                for t in range(3):
                    for which in range(2):
                        wconv(ru, t, which)
            return carry

        lax.fori_loop(0, NR, ph1, 0)

        def fft16(g8, t, sign, emit):
            lr = []
            li = []
            for a in range(16):
                r0 = pl.multiple_of(a * 128 + g8 * 8, 8)
                lr.append(xr[t, pl.ds(r0, 8), :])
                li.append(xi[t, pl.ds(r0, 8), :])
            yr, yi = _fft_list(lr, li, sign)
            for a in range(16):
                emit(a, pl.multiple_of(a * 128 + g8 * 8, 8), yr[a], yi[a])

        def emit_f32(t):
            def f(a, r0, re, im):
                fr[t, pl.ds(r0, 8), :] = re
                fi[t, pl.ds(r0, 8), :] = im
            return f

        wqkv_cp.wait()
        wt[0:D, :] = wqkv_v[:, 0:D].T
        wt[D:2 * D, :] = wqkv_v[:, 2 * D:3 * D].T
        bx_cp.wait()

        def ph2(r, carry):
            r0 = pl.multiple_of(r * 512, 512)
            x = bx_v[:, pl.ds(r0, 512)]
            PR = 96
            NP = 2 * D // PR
            for u in range(NP):
                y = jnp.dot(wt[u * PR:(u + 1) * PR, :], x, preferred_element_type=F32)
                if u < NP // 2:
                    yq = (y * scale).astype(BF16)
                    qp[u * PR // 2:(u + 1) * PR // 2, pl.ds(r0, 512)] = pltpu.bitcast(yq, jnp.uint32)
                    qf[u * PR:(u + 1) * PR, pl.ds(r0, 512)] = yq.astype(F32)
                else:
                    vt[u * PR - D:(u + 1) * PR - D, pl.ds(r0, 512)] = y.astype(BF16).astype(F32)
                fft16(r * 4 + u // 3, u % 3, -1, emit_f32(u % 3))
            return carry

        lax.fori_loop(0, NR, ph2, 0)

        rows8 = lax.broadcasted_iota(jnp.int32, (8, 512), 0)
        zero8 = jnp.zeros((8, 512), jnp.uint32)
        rows8v = lax.broadcasted_iota(jnp.int32, (8, 512), 0)

        def mkq(h, r):
            _, fa, fb = _head_tile(h)
            plo, phi = h * DH // 2, (h * DH + DH) // 2
            c0 = pl.multiple_of(r * 512, 512)
            parts = []
            for v in range(8):
                p0 = (fa if v < 4 else fb) // 2 + 8 * (v % 4)
                if p0 + 8 <= plo or p0 >= phi:
                    parts.append(zero8)
                else:
                    w = qp[p0:p0 + 8, pl.ds(c0, 512)]
                    if not (p0 >= plo and p0 + 8 <= phi):
                        w = jnp.where((rows8 >= plo - p0) & (rows8 < phi - p0), w, zero8)
                    parts.append(w)
            w = jnp.concatenate(parts, axis=0)
            for n in range(4):
                qm[h, r * 4 + n] = w[:, n * 128:(n + 1) * 128]

        def mkv(h, r):
            lo = h * DH
            w0 = lo // 8 * 8
            o = lo - w0
            ones_row = 0 if o == 6 else 23
            c0 = pl.multiple_of(r * 512, 512)
            for v in range(3):
                win = vt[w0 + 8 * v:w0 + 8 * v + 8, pl.ds(c0, 512)]
                fill = jnp.where(rows8v == ones_row - 8 * v, 1.0, 0.0)
                vtp[h, 8 * v:8 * v + 8, pl.ds(c0, 512)] = jnp.where(
                    (rows8v >= o - 8 * v) & (rows8v < o + DH - 8 * v), win, fill)

        g_cp.wait()
        gi_cp.wait()

        def ph3(r, carry):
            def fwd(k1):
                r0 = pl.multiple_of(k1 * 128, 128)
                st = jnp.concatenate(
                    [jnp.concatenate([fr[t, pl.ds(r0, 128), :] for t in range(3)], axis=1),
                     jnp.concatenate([fi[t, pl.ds(r0, 128), :] for t in range(3)], axis=1)], axis=0).astype(BF16)
                return jnp.dot(g_v[k1], st, preferred_element_type=F32)

            def inv(k1, o):
                r0 = pl.multiple_of(k1 * 128, 128)
                orr = o[0:128]
                oi = o[128:256]
                wr = jnp.concatenate([wrf[t, pl.ds(k1, 128, stride=16), :] for t in range(3)], axis=1)
                wi = jnp.concatenate([wif[t, pl.ds(k1, 128, stride=16), :] for t in range(3)], axis=1)
                zr = orr * wr - oi * wi
                zi = orr * wi + oi * wr
                z = jnp.concatenate([zr, zi], axis=0).astype(BF16)
                u = jnp.dot(gi_v[k1], z, preferred_element_type=F32)
                for t in range(3):
                    xr[t, pl.ds(r0, 128), :] = u[0:128, t * 128:(t + 1) * 128]
                    xi[t, pl.ds(r0, 128), :] = u[128:256, t * 128:(t + 1) * 128]

            o = fwd(r * 4)
            for u in range(4):
                on = fwd(r * 4 + u + 1) if u < 3 else None
                for h in range(8 * u, 8 * u + 4):
                    mkq(h, r)
                inv(r * 4 + u, o)
                for h in range(8 * u + 4, 8 * u + 8):
                    mkq(h, r)
                o = on
            return carry

        lax.fori_loop(0, 4, ph3, 0)

        lane = lax.broadcasted_iota(jnp.int32, (128, 128), 1)
        lane8 = lax.broadcasted_iota(jnp.int32, (8, 128), 1)

        def emit_ul(t):
            def f(a, r0, re, im):
                if t < 2:
                    ul[t, pl.ds(r0, 8), :] = re
                    ul[2 + t, pl.ds(r0, 8), :] = im
                else:
                    ul[4, pl.ds(r0, 8), :] = jnp.where(lane8 < 64, re, pltpu.roll(im, 64, 1))
            return f

        def ph4(r, carry):
            for u in range(4):
                ru = pl.multiple_of(r * 512 + u * 128, 128)
                kk = lax.dot_general(bx_v[:, pl.ds(ru, 128)], wqkv_v[:, 512:1152], TN,
                                     preferred_element_type=F32).astype(BF16)
                for t in range(5):
                    kt[t, pl.ds(ru, 128), :] = kk[:, 128 * t:128 * (t + 1)]
                for j in range(4):
                    kt[5 + j, pl.ds(ru, 128), :] = jnp.where(
                        lane >= 64, kk[:, 128 * j:128 * (j + 1)], kk[:, 128 * (j + 1):128 * (j + 2)])
                for v in range(3):
                    fft16(r * 4 + u, v, +1, emit_ul(v))
                    for h in range(8 * u + 3 * v, min(8 * u + 3 * v + 3, 8 * u + 8)):
                        mkv(h, r)
            return carry

        lax.fori_loop(0, NR, ph4, 0)
        for h in range(H):
            tile, fa, fb = _head_tile(h)
            lo = h * DH
            l0 = (lo - fa) if fa <= lo < fa + 64 else (lo - fb + 64)
            kv[h] = pltpu.roll(kt[tile, 0:128 * NV, :].astype(F32), (128 - l0) % 128, 1)
        wo_cp.wait()
        fdi_cp.wait()

    rows128 = lax.broadcasted_iota(jnp.int32, (128, 128), 0)

    def getq(h, qb):
        return jnp.concatenate([pltpu.bitcast(qm[h, qb * NT + n], BF16) for n in range(NT)], axis=1)

    def ktile(h):
        lo = h * DH
        j = lo >> 7
        straddle = (((lo + DH - 1) >> 7) != j) | (j == 4)
        return jnp.where(straddle, (lo + 64) >> 7, 5 + j)

    rows24 = lax.broadcasted_iota(jnp.int32, (24, 128), 0)

    def finish_piece(h0, oraw, g, n):
        cols = slice(n * 128, (n + 1) * 128)
        o = oraw[g, :, cols]
        lo = (h0 + g) * DH
        w0 = pl.multiple_of((lo >> 3) << 3, 8)
        off = lo - w0
        l = jnp.where(off == 6, o[0:1, :], o[23:24, :])
        val = o * (1.0 / l)
        msk = (rows24 >= off) & (rows24 < off + DH)
        ot[pl.ds(w0, 24), cols] = jnp.where(msk, val, ot[pl.ds(w0, 24), cols])

    def finish(h0, oraw):
        for g in range(G):
            for n in range(NT):
                finish_piece(h0, oraw, g, n)

    def bcast_q(slot, h, qb, d):
        q0 = pl.multiple_of(qb * QB, QB)
        qbt[slot, d] = jnp.broadcast_to(qf[pl.ds(h * DH + d, 1), pl.ds(q0, QB)], (8, QB))

    def step(h_next, qb_next, s_next, m_next, h_cur, s_cur, m_cur, o_cur, do_next, do_cur, fin=None, nxt=None):
        cs = []
        ms = []
        for g in range(G):
            if do_next:
                cs.append(ktile(h_next + g))
        for g in range(G):
            if do_cur:
                ms.append(jnp.max(m_cur[g], axis=0, keepdims=True))
            mx = None
            o = None
            for j in range(NCH):
                if do_next and j != SK:
                    jj = j + 1 if j < SK else j
                    s = jnp.dot(kt[cs[g], pl.ds(jj * CH, CH), :], getq(h_next + g, qb_next), preferred_element_type=F32)
                    s_next[g][pl.ds(jj * CH, CH), :] = s
                    sm = jnp.max(s.reshape(CH // 8, 8, QB), axis=0)
                    mx = sm if mx is None else jnp.maximum(mx, sm)
                if do_next and 2 <= j < 11 and (g == 0 or nxt is not None):
                    hh, qq = (h_next + 1, qb_next) if g == 0 else nxt
                    for d in (2 * (j - 2), 2 * (j - 2) + 1):
                        bcast_q(1 - g, hh, qq, d)
                def vpu_part(mx):
                    nk = 16 * NV
                    span = NCH
                    for kg in range(j * nk // span, (j + 1) * nk // span):
                        kvv = kv[h_next + g, kg * 8:(kg + 1) * 8, :]
                        acc = None
                        for d in range(DH):
                            t = kvv[:, d:d + 1] * qbt[g, d]
                            acc = t if acc is None else acc + t
                        s_next[g][kg * 8:(kg + 1) * 8, :] = acc
                        mx = acc if mx is None else jnp.maximum(mx, acc)
                    return mx

                if do_next:
                    mx = vpu_part(mx)
                if do_cur:
                    p = jnp.exp2(s_cur[g][pl.ds(j * CH, CH), :] - ms[g]).astype(BF16)
                    d = jnp.dot(vtp[h_cur + g, :, pl.ds(j * CH, CH)], p, preferred_element_type=F32)
                    o = d if o is None else o + d
                if g == 0 and 3 <= j < 3 + G * NT and fin is not None:
                    finish_piece(fin[0], fin[1], (j - 3) // NT, (j - 3) % NT)
            if do_cur:
                o_cur[g] = o
            if do_next:
                m_next[g] = mx

    SA = (sa0, sa1)
    SB = (sb0, sb1)

    @pl.when(i == 0)
    def _prologue():
        for d in range(DH):
            bcast_q(0, 0, 0, d)
        step(0, 0, SA, ma, 0, None, None, None, True, False, nxt=(G, 0))

    def pair(n, last_pair):
        for par in range(2):
            st = 2 * n + par
            h_cur = st * G
            h_next = jnp.where(st == NSTEP - 1, 0, h_cur + G)
            qb_next = jnp.where(st == NSTEP - 1, jnp.minimum(i + 1, NQB - 1), i)
            h_fin = jnp.maximum(h_cur - G, 0)
            wrap = st >= NSTEP - 2
            nxt = (jnp.where(wrap, h_cur + 2 * G - H, h_cur + 2 * G), jnp.where(wrap, jnp.minimum(i + 1, NQB - 1), i))
            if par == 0:
                step(h_next, qb_next, SB, mb, h_cur, SA, ma, ora, True, True, fin=(h_fin, orb), nxt=nxt)
            elif not last_pair:
                step(h_next, qb_next, SA, ma, h_cur, SB, mb, orb, True, True, fin=(h_fin, ora), nxt=nxt)
            else:
                step(h_next, qb_next, SA, ma, h_cur, SB, mb, orb, False, True, fin=(h_fin, ora))

    def body(n, carry):
        very_last = (n == NSTEP // 2 - 1) & (i == NQB - 1)

        @pl.when(jnp.logical_not(very_last))
        def _():
            pair(n, False)

        @pl.when(very_last)
        def _():
            pair(n, True)

        return carry

    lax.fori_loop(0, NSTEP // 2, body, 0)
    finish(H - G, orb)

    r0 = pl.multiple_of(i * QB, QB)
    ua = jnp.concatenate([ul[t, pl.ds(r0, QB), :] for t in range(5)], axis=1).astype(BF16)
    ya = jnp.dot(ua, fdi_v[...], preferred_element_type=F32)
    out_ref[:, 0:D] = ya.astype(BF16)
    yb = lax.dot_general(ot[...].astype(BF16), wo_v[...], (((0,), (0,)), ((), ())), preferred_element_type=F32)
    out_ref[:, D:2 * D] = yb.astype(BF16)


@jax.jit
def pallas_concat_heads__spectral_gfnet__mha_block__prompt_kernel(
    A_x: jax.Array,
    A_w_r: jax.Array,
    A_w_i: jax.Array,
    B_x: jax.Array,
    B_wqkv: jax.Array,
    B_wo: jax.Array,
):
    ax = A_x.reshape(S, D).T
    bx = B_x.reshape(S, D).T
    fd = jnp.asarray(_FD).astype(BF16)
    fdi = jnp.asarray(_FDI).astype(BF16)
    g = jnp.asarray(_G).astype(BF16)
    gi = jnp.asarray(_GI).astype(BF16)
    any_spec = pl.BlockSpec(memory_space=pl.ANY)
    VM = pltpu.VMEM
    scratch = [
        VM((D, S), BF16), VM((DF, S), BF16), VM((DF, S), BF16), VM((D, S), BF16),
        VM((D, 3 * D), BF16), VM((D, D), BF16), VM((D, 640), BF16), VM((640, D), BF16),
        VM((16, 256, 256), BF16), VM((16, 256, 256), BF16), pltpu.SemaphoreType.DMA((19,)),
        VM((9, S, 128), BF16), VM((H, S // 128, 64, 128), jnp.uint32), VM((D // 2, S), jnp.uint32), VM((D, S), F32), VM((H, 128 * NV, 128), F32), VM((G, DH, 8, QB), F32), VM((D, S), F32), VM((H, 24, S), F32), VM((2 * D, D), BF16),
        VM((3, S, 128), F32), VM((3, S, 128), F32), VM((3, S, 128), F32), VM((3, S, 128), F32), VM((3, S, 128), F32), VM((3, S, 128), F32), VM((5, S, 128), F32),
        VM((S, QB), F32), VM((S, QB), F32), VM((S, QB), F32), VM((S, QB), F32),
        VM((G, 8, QB), F32), VM((G, 8, QB), F32),
        VM((D, QB), F32), VM((G, 24, QB), F32), VM((G, 24, QB), F32),
    ]
    out = pl.pallas_call(
        _kernel,
        grid=(NQB,),
        in_specs=[any_spec] * 10,
        out_specs=pl.BlockSpec((QB, 2 * D), lambda i: (i, 0)),
        out_shape=jax.ShapeDtypeStruct((S, 2 * D), BF16),
        scratch_shapes=scratch,
        compiler_params=pltpu.CompilerParams(
            dimension_semantics=("arbitrary",), vmem_limit_bytes=120 * 1024 * 1024),
        name="mha_gfnet",
    )(ax, A_w_r.T, A_w_i.T, bx, B_wqkv, B_wo, fd, fdi, g, gi)
    return out.reshape(1, S, 2 * D)
```
